```python
import jax
import jax.numpy as jnp

def _softmax(x, axis=-1):
    return jax.nn.softmax(x, axis=axis)
def _gelu(x):
    return jax.nn.gelu(x, approximate=True)
def _silu(x):
    return jax.nn.silu(x)
def _sigmoid(x):
    return jax.nn.sigmoid(x)
def _layernorm(x, axis=-1, eps=1e-5):
    m = jnp.mean(x, axis=axis, keepdims=True)
    v = jnp.var(x, axis=axis, keepdims=True)
    return (x - m) / jnp.sqrt(v + eps)
def _scatter_add(tgt, idx, src, axis=0):
    return tgt.at[idx].add(src)
def _segment_sum(src, seg, n):
    return jax.ops.segment_sum(src, seg, n)
class _Rng:
    def __init__(self, key):
        self._k = key
    def _next(self):
        self._k, sub = jax.random.split(self._k)
        return sub
    def normal(self, shape):
        return jax.random.normal(self._next(), shape, dtype=jnp.bfloat16)
    def randint(self, lo, hi, shape):
        return jax.random.randint(self._next(), shape, lo, hi, dtype=jnp.int32)
    def uniform(self, shape, lo=0.0, hi=1.0):
        return jax.random.uniform(self._next(), shape, jnp.bfloat16, lo, hi)
    def permutation(self, n):
        return jax.random.permutation(self._next(), n)


kernel_name = 'gated_mix__compressed_kv_cla__sliding_block_cached__decode'

def setup_inputs():
    _rng = _Rng(jax.random.key(int.from_bytes(__import__("os").urandom(4), "little")))
    _w = (lambda a: (lambda t: t.astype(jnp.bfloat16) if jnp.issubdtype(t.dtype, jnp.floating) else t)(jnp.asarray(a)))
    def _A_setup():
        B, H, Sq, Sk, D, M = 8, 32, 1, 4096, 128, 512
        Dc = 4 * D
        return {
            "x": _w((lambda *s: _rng.normal(s) * 0.05)(B, Sq, M)),
            "c_kv": _w((lambda *s: _rng.normal(s) * 0.05)(B, Sk, Dc)),
            "w_q": _w((lambda *s: _rng.normal(s) * 0.05)(M, H, D) * (M ** -0.5)),
            "w_uk": _w((lambda *s: _rng.normal(s) * 0.05)(Dc, H, D) * (Dc ** -0.5)),
            "w_uv": _w((lambda *s: _rng.normal(s) * 0.05)(Dc, H, D) * (Dc ** -0.5)),
            "w_o": _w((lambda *s: _rng.normal(s) * 0.05)(H, D, M) * ((H * D) ** -0.5)),
        }
    _A_in = _A_setup()

    def _B_setup():
        B, Sq, D = 8, 1, 512
        Hq, Hkv, Sk, Dh = 32, 8, 4096, 128
        assert Hq % Hkv == 0, (Hq, Hkv)
        return {
            "x": _w((lambda *s: _rng.normal(s) * 0.05)(B, Sq, D)),
            "k_cache": _w((lambda *s: _rng.normal(s) * 0.05)(B, Hkv, Sk, Dh)),
            "v_cache": _w((lambda *s: _rng.normal(s) * 0.05)(B, Hkv, Sk, Dh)),
            "wq": _w((lambda *s: _rng.normal(s) * 0.05)(D, Hq * Dh) * (D ** -0.5)),
            "wo": _w((lambda *s: _rng.normal(s) * 0.05)(Hq * Dh, D) * ((Hq * Dh) ** -0.5)),
        }
    _B_in = _B_setup()

    return {
        "A_x": _A_in["x"],
        "A_c_kv": _A_in["c_kv"],
        "A_w_q": _A_in["w_q"],
        "A_w_uk": _A_in["w_uk"],
        "A_w_uv": _A_in["w_uv"],
        "A_w_o": _A_in["w_o"],
        "B_x": _B_in["x"],
        "B_k_cache": _B_in["k_cache"],
        "B_v_cache": _B_in["v_cache"],
        "B_wq": _B_in["wq"],
        "B_wo": _B_in["wo"],
        "gate_w": _w((lambda *s: _rng.normal(s) * 0.05)(512)),
    }

def reference(A_x, A_c_kv, A_w_q, A_w_uk, A_w_uv, A_w_o, B_x, B_k_cache, B_v_cache, B_wq, B_wo, gate_w):
    def _A_ref(x, c_kv, w_q, w_uk, w_uv, w_o):
        B, Sq, M = x.shape[0], x.shape[1], x.shape[2]
        Sk = c_kv.shape[1]
        H, D = w_q.shape[1], w_q.shape[2]
        q = jnp.einsum("bqm,mhd->bhqd", x, w_q)
        k = jnp.einsum("bkc,chd->bhkd", c_kv, w_uk)
        v = jnp.einsum("bkc,chd->bhkd", c_kv, w_uv)
        scores = jnp.einsum("bhqd,bhkd->bhqk", q, k) * (D ** -0.5)
        off = Sk - Sq
        qi = jnp.arange(Sq)[:, None]
        kj = jnp.arange(Sk)[None, :]
        cmask = kj <= (qi + off)
        scores = jnp.where(cmask[None, None], scores, -1e9)
        p = _softmax(scores, axis=-1)
        ctx = jnp.einsum("bhqk,bhkd->bhqd", p, v)
        return jnp.einsum("bhqd,hdm->bqm", ctx, w_o)

    def _B_ref(x, k_cache, v_cache, wq, wo):
        B, Sq, D = x.shape
        Hq, Dh = 32, 128
        Hkv, Sk = k_cache.shape[1], k_cache.shape[2]
        W = min(4096, max(256, Sk // 4))
        rep = Hq // Hkv
        q = (lambda x, *d: x.transpose(*d))((x @ wq).reshape(B, Sq, Hq, Dh), 0, 2, 1, 3)
        k = jnp.repeat(k_cache[:, :, Sk - W:, :], rep, axis=1)
        v = jnp.repeat(v_cache[:, :, Sk - W:, :], rep, axis=1)
        scores = jnp.einsum("bhqd,bhkd->bhqk", q, k) * (Dh ** -0.5)
        p = _softmax(scores, axis=-1)
        o = jnp.einsum("bhqk,bhkd->bhqd", p, v)
        return (lambda x, *d: x.transpose(*d))(o, 0, 2, 1, 3).reshape(B, Sq, Hq * Dh) @ wo

    x = A_x
    g = _sigmoid((x * gate_w).sum(-1, keepdims=True))
    a = _A_ref(x, A_c_kv, A_w_q, A_w_uk, A_w_uv, A_w_o)
    b = _B_ref(x, B_k_cache, B_v_cache, B_wq, B_wo)
    return g * a + (1 - g) * b
```

```python
import jax
import jax.numpy as jnp
from jax import lax
import jax.experimental.pallas as pl
import jax.experimental.pallas.tpu as pltpu

MiB = 1 << 20
BF = jnp.bfloat16
F32 = jnp.float32
U32 = jnp.uint32
NN = (((1,), (0,)), ((), ()))
NT = (((1,), (1,)), ((), ()))

B, H, D, M, DC, SK = 8, 32, 128, 512, 512, 4096
HKV, W = 8, 1024
SCALE = D ** -0.5

CKV_GROUPS = (4, 4)
KV_GROUPS = (4, 3, 1)
WO_CHUNKS = (16, 12, 4)


def _dot(a, b, dims=NN):
    return lax.dot_general(a, b, dims, preferred_element_type=F32)


def _head_pair(w32, h2):
    a = w32[pl.ds(h2, 256, stride=32), :]
    b = w32[pl.ds(h2 + 16, 256, stride=32), :]
    lo = (a & jnp.uint32(0xFFFF)) | (b << 16)
    hi = (a >> 16) | (b & jnp.uint32(0xFFFF0000))
    return pltpu.bitcast(lo, BF), pltpu.bitcast(hi, BF)


def _kernel(x_hbm, ckv_hbm, wq_hbm, wuk_hbm, wuv_hbm, wo_hbm, bx_hbm, k_hbm, v_hbm, bwq_hbm, bwo_hbm, g_hbm,
            out_ref,
            x_v, bx_v, g_v, ckv_v, wq_v, wuk_v, wuv_v, wo_v, k_v, v_v, bwq_v, bwo_v,
            qlat_s, qb_s, ql_v, qblk_v, s_s, cl_s, o_s, ob_v, sems):
    cp = pltpu.make_async_copy
    g_w1 = [cp(wq_hbm, wq_v, sems.at[0]), cp(wuk_hbm, wuk_v, sems.at[0]), cp(bwq_hbm, bwq_v, sems.at[0]),
            cp(x_hbm, x_v, sems.at[0]), cp(bx_hbm, bx_v, sems.at[0]), cp(g_hbm, g_v, sems.at[0])]
    si = 1
    g_ckv = []
    b0 = 0
    for n in CKV_GROUPS:
        g_ckv.append((b0, [cp(ckv_hbm.at[pl.ds(b0, n)], ckv_v.at[pl.ds(b0, n)], sems.at[si])]))
        b0 += n
        si += 1
    g_w2 = [cp(wuv_hbm, wuv_v, sems.at[si]), cp(wo_hbm, wo_v, sems.at[si])]
    si += 1
    g_kv = []
    b0 = 0
    for n in KV_GROUPS:
        g_kv.append((b0, [
            cp(k_hbm.at[pl.ds(b0, n), :, pl.ds(SK - W, W)], k_v.at[pl.ds(b0, n)], sems.at[si]),
            cp(v_hbm.at[pl.ds(b0, n), :, pl.ds(SK - W, W)], v_v.at[pl.ds(b0, n)], sems.at[si])]))
        b0 += n
        si += 1
    g_wo = []
    h0 = 0
    for n in WO_CHUNKS:
        g_wo.append((h0, n, [cp(bwo_hbm.at[pl.ds(h0 * D, n * D)], bwo_v.at[pl.ds(h0 * D, n * D)], sems.at[si])]))
        h0 += n
        si += 1

    def start(g):
        for c in g:
            c.start()

    def wait(g):
        for c in g:
            c.wait()

    start(g_w1)
    for _, g in g_ckv:
        start(g)
    start(g_w2)
    for _, g in g_kv:
        start(g)
    for _, _, g in g_wo:
        start(g)

    wait(g_w1)
    x = x_v[...]
    bx = bx_v[...]
    wq32 = wq_v.bitcast(U32)
    wuk32 = wuk_v.bitcast(U32)
    for h2 in range(H // 2):
        wq_pair = _head_pair(wq32, h2)
        wk_pair = _head_pair(wuk32, h2)
        for p in range(2):
            h = 2 * h2 + p
            q = _dot(x, wq_pair[p])
            ql = _dot(q.astype(BF), wk_pair[p], NT)
            for cc in range(4):
                qlat_s[pl.ds(cc * 256 + h * 8, 8), :] = ql[:, cc * 128:(cc + 1) * 128]
    for j in range(8):
        qb = _dot(bx, bwq_v[:, j * 512:(j + 1) * 512])
        for r in range(4):
            qb_s[pl.ds((j * 4 + r) * 8, 8), :] = qb[:, r * 128:(r + 1) * 128]
    row16 = lax.broadcasted_iota(jnp.int32, (16, 128), 0)
    for b in range(B):
        parts = [qlat_s[pl.ds(cc * 256 + b, H, stride=8), :] for cc in range(4)]
        ql_v[b] = jnp.concatenate(parts, axis=1).astype(BF)
        qb = qb_s[pl.ds(b, H, stride=8), :]
        for half in range(2):
            qh = qb[half * 16:(half + 1) * 16, :]
            blk = [jnp.where((row16 >= 4 * gi) & (row16 < 4 * gi + 4), qh, 0.0) for gi in range(4)]
            qblk_v[b, half] = jnp.concatenate(blk, axis=1).astype(BF)
    gw = g_v[...].astype(F32).reshape(1, M)
    gate = jax.nn.sigmoid(jnp.sum(x.astype(F32) * gw, axis=-1, keepdims=True))

    T = 1024

    def a_body(b, carry):
        for b0, g in g_ckv:
            @pl.when(b == b0)
            def _():
                wait(g)
        q = ql_v[b]
        mx = None
        for j in range(SK // T):
            s = _dot(q, ckv_v[b, pl.ds(j * T, T), :], NT) * SCALE
            s_s[:, pl.ds(j * T, T)] = s
            for t in range(T // 128):
                blk = s[:, t * 128:(t + 1) * 128]
                mx = blk if mx is None else jnp.maximum(mx, blk)
        m = jnp.max(mx, axis=-1, keepdims=True)
        l = jnp.zeros((H, 128), F32)
        acc = jnp.zeros((H, DC), F32)
        for j in range(SK // T):
            p = jnp.exp(s_s[:, pl.ds(j * T, T)] - m)
            for t in range(T // 128):
                l = l + p[:, t * 128:(t + 1) * 128]
            acc = acc + _dot(p.astype(BF), ckv_v[b, pl.ds(j * T, T), :])
        o = acc / jnp.sum(l, axis=-1, keepdims=True)
        for cc in range(4):
            cl_s[pl.ds(pl.multiple_of(cc * 256 + b * 32, 32), 32), :] = o[:, cc * 128:(cc + 1) * 128]
        return carry

    lax.fori_loop(0, B, a_body, 0)

    wait(g_w2)
    wuv32 = wuv_v.bitcast(U32)
    out_a = jnp.zeros((B, M), F32)
    for h2 in range(H // 2):
        wv_pair = _head_pair(wuv32, h2)
        for p in range(2):
            h = 2 * h2 + p
            cl = jnp.concatenate([cl_s[pl.ds(cc * 256 + h, B, stride=32), :] for cc in range(4)], axis=1)
            ctx = _dot(cl.astype(BF), wv_pair[p])
            out_a = out_a + _dot(ctx.astype(BF), wo_v[pl.ds(h * D, D), :])

    def b_body(b, carry):
        for b0, g in g_kv:
            @pl.when(b == b0)
            def _():
                wait(g)
        for half in range(2):
            kcat = jnp.concatenate([k_v[b, half * 4 + gi] for gi in range(4)], axis=1)
            s = _dot(qblk_v[b, half], kcat, NT) * SCALE
            m = jnp.max(s, axis=-1, keepdims=True)
            p = jnp.exp(s - m)
            l = jnp.sum(p, axis=-1, keepdims=True)
            pb = p.astype(BF)
            o = None
            for gi in range(4):
                og = _dot(pb, v_v[b, half * 4 + gi])
                o = og if o is None else jnp.where(row16 >= 4 * gi, og, o)
            o_s[pl.ds(pl.multiple_of(b * 32 + half * 16, 16), 16), :] = o / l
        return carry

    lax.fori_loop(0, B, b_body, 0)
    for h in range(H):
        ob_v[:, pl.ds(h * D, D)] = o_s[pl.ds(h, B, stride=32), :].astype(BF)
    out_b = jnp.zeros((B, M), F32)
    for h0, n, g in g_wo:
        wait(g)
        out_b = out_b + _dot(ob_v[:, pl.ds(h0 * D, n * D)], bwo_v[pl.ds(h0 * D, n * D), :])
    out_ref[...] = (gate * out_a + (1.0 - gate) * out_b).astype(out_ref.dtype)


@jax.jit
def pallas_gated_mix__compressed_kv_cla__sliding_block_cached__decode_kernel(
    A_x: jax.Array,
    A_c_kv: jax.Array,
    A_w_q: jax.Array,
    A_w_uk: jax.Array,
    A_w_uv: jax.Array,
    A_w_o: jax.Array,
    B_x: jax.Array,
    B_k_cache: jax.Array,
    B_v_cache: jax.Array,
    B_wq: jax.Array,
    B_wo: jax.Array,
    gate_w: jax.Array,
):
    n_sems = 1 + len(CKV_GROUPS) + 1 + len(KV_GROUPS) + len(WO_CHUNKS)
    out = pl.pallas_call(
        _kernel,
        in_specs=[pl.BlockSpec(memory_space=pl.ANY)] * 12,
        out_specs=pl.BlockSpec(memory_space=pltpu.VMEM),
        out_shape=jax.ShapeDtypeStruct((B, M), BF),
        scratch_shapes=[
            pltpu.VMEM((B, M), BF), pltpu.VMEM((B, M), BF), pltpu.VMEM((M,), BF),
            pltpu.VMEM((B, SK, DC), BF),
            pltpu.VMEM((M * H, D), BF), pltpu.VMEM((DC * H, D), BF), pltpu.VMEM((DC * H, D), BF),
            pltpu.VMEM((H * D, M), BF),
            pltpu.VMEM((B, HKV, W, D), BF), pltpu.VMEM((B, HKV, W, D), BF),
            pltpu.VMEM((M, H * D), BF), pltpu.VMEM((H * D, M), BF),
            pltpu.VMEM((4 * 256, 128), F32), pltpu.VMEM((256, 128), F32),
            pltpu.VMEM((B, H, DC), BF), pltpu.VMEM((B, 2, 16, 512), BF),
            pltpu.VMEM((H, SK), F32), pltpu.VMEM((4 * 256, 128), F32),
            pltpu.VMEM((256, 128), F32), pltpu.VMEM((B, H * D), BF),
            pltpu.SemaphoreType.DMA((n_sems,)),
        ],
        compiler_params=pltpu.CompilerParams(vmem_limit_bytes=100 * MiB),
    )(A_x.reshape(B, M), A_c_kv, A_w_q.reshape(M * H, D), A_w_uk.reshape(DC * H, D), A_w_uv.reshape(DC * H, D),
      A_w_o.reshape(H * D, M), B_x.reshape(B, M), B_k_cache, B_v_cache, B_wq, B_wo, gate_w)
    return out.reshape(B, 1, M)
```

```python
import jax
import jax.numpy as jnp
from jax import lax
import jax.experimental.pallas as pl
import jax.experimental.pallas.tpu as pltpu

MiB = 1 << 20
BF = jnp.bfloat16
F32 = jnp.float32
U32 = jnp.uint32
NN = (((1,), (0,)), ((), ()))
NT = (((1,), (1,)), ((), ()))

B, H, D, M, DC, SK = 8, 32, 128, 512, 512, 4096
HKV, W = 8, 1024
SCALE = D ** -0.5

KV_GROUPS = (4, 3, 1)
WO_HEAD = 16
N_TAIL = H - WO_HEAD
N_SEMS = 1 + len(KV_GROUPS) + 1 + N_TAIL


def _dot(a, b, dims=NN):
    return lax.dot_general(a, b, dims, preferred_element_type=F32)


def _head_pair(w32, h2):
    a = w32[pl.ds(h2, 256, stride=32), :]
    b = w32[pl.ds(h2 + 16, 256, stride=32), :]
    lo = (a & jnp.uint32(0xFFFF)) | (b << 16)
    hi = (a >> 16) | (b & jnp.uint32(0xFFFF0000))
    return pltpu.bitcast(lo, BF), pltpu.bitcast(hi, BF)


def _kernel(x_hbm, ckv_hbm, wq_hbm, wuk_hbm, wuv_hbm, wo_hbm, bx_hbm, k_hbm, v_hbm, bwq_hbm, bwo_hbm, g_hbm,
            out_hbm,
            x_v, bx_v, g_v, ckv_v, wq_v, wuk_v, wuv_v, wo_v, k_v, v_v, bwq_v, bwo_v,
            qlat_s, qb_s, ql_v, qblk_v, s_s, cl_s, o_s, ob_v, out_v, out_sem):
    cp = pltpu.make_async_copy
    out_copy = cp(out_v, out_hbm, out_sem)

    def body(sems):
        g_a = [cp(wq_hbm, wq_v, sems.at[0]), cp(wuk_hbm, wuk_v, sems.at[0]), cp(bwq_hbm, bwq_v, sems.at[0]),
               cp(x_hbm, x_v, sems.at[0]), cp(bx_hbm, bx_v, sems.at[0]), cp(g_hbm, g_v, sems.at[0]),
               cp(ckv_hbm, ckv_v, sems.at[0])]
        g_kv = []
        b0 = 0
        for i, n in enumerate(KV_GROUPS):
            sem = sems.at[1 + i]
            g = [cp(k_hbm.at[pl.ds(b0, n), :, pl.ds(SK - W, W)], k_v.at[pl.ds(b0, n)], sem),
                 cp(v_hbm.at[pl.ds(b0, n), :, pl.ds(SK - W, W)], v_v.at[pl.ds(b0, n)], sem)]
            if i == 0:
                g = [cp(wuv_hbm, wuv_v, sem), cp(wo_hbm, wo_v, sem)] + g
            g_kv.append((b0, g))
            b0 += n
        sem_wo = 1 + len(KV_GROUPS)
        g_wo = [cp(bwo_hbm.at[pl.ds(0, WO_HEAD * D)], bwo_v.at[pl.ds(0, WO_HEAD * D)], sems.at[sem_wo])]

        def tail_copy(c):
            off = pl.multiple_of((WO_HEAD + c) * D, D)
            return cp(bwo_hbm.at[pl.ds(off, D)], bwo_v.at[pl.ds(off, D)], sems.at[sem_wo + 1 + c])

        def start(g):
            for c in g:
                c.start()

        def wait(g):
            for c in g:
                c.wait()

        start(g_a)
        for _, g in g_kv:
            start(g)
        start(g_wo)
        start([tail_copy(c) for c in range(N_TAIL)])

        wait(g_a)
        x = x_v[...]
        bx = bx_v[...]
        wq32 = wq_v.bitcast(U32)
        wuk32 = wuk_v.bitcast(U32)
        for h2 in range(H // 2):
            wq_pair = _head_pair(wq32, h2)
            wk_pair = _head_pair(wuk32, h2)
            for p in range(2):
                h = 2 * h2 + p
                q = _dot(x, wq_pair[p])
                ql = _dot(q.astype(BF), wk_pair[p], NT)
                for cc in range(4):
                    qlat_s[pl.ds(cc * 256 + h * 8, 8), :] = ql[:, cc * 128:(cc + 1) * 128]
        for j in range(8):
            qb = _dot(bx, bwq_v[:, j * 512:(j + 1) * 512])
            for r in range(4):
                qb_s[pl.ds((j * 4 + r) * 8, 8), :] = qb[:, r * 128:(r + 1) * 128]
        row16 = lax.broadcasted_iota(jnp.int32, (16, 128), 0)
        for b in range(B):
            parts = [qlat_s[pl.ds(cc * 256 + b, H, stride=8), :] for cc in range(4)]
            ql_v[b] = jnp.concatenate(parts, axis=1).astype(BF)
            qb = qb_s[pl.ds(b, H, stride=8), :]
            for half in range(2):
                qh = qb[half * 16:(half + 1) * 16, :]
                blk = [jnp.where((row16 >= 4 * gi) & (row16 < 4 * gi + 4), qh, 0.0) for gi in range(4)]
                qblk_v[b, half] = jnp.concatenate(blk, axis=1).astype(BF)
        gw = g_v[...].astype(F32).reshape(1, M)
        gate = jax.nn.sigmoid(jnp.sum(x.astype(F32) * gw, axis=-1, keepdims=True))

        T = 1024

        def a_body(b, carry):
            q = ql_v[b]
            mx = None
            for j in range(SK // T):
                s = _dot(q, ckv_v[b, pl.ds(j * T, T), :], NT) * SCALE
                s_s[:, pl.ds(j * T, T)] = s
                for t in range(T // 128):
                    blk = s[:, t * 128:(t + 1) * 128]
                    mx = blk if mx is None else jnp.maximum(mx, blk)
            m = jnp.max(mx, axis=-1, keepdims=True)
            l = jnp.zeros((H, 128), F32)
            acc = jnp.zeros((H, DC), F32)
            for j in range(SK // T):
                p = jnp.exp(s_s[:, pl.ds(j * T, T)] - m)
                for t in range(T // 128):
                    l = l + p[:, t * 128:(t + 1) * 128]
                acc = acc + _dot(p.astype(BF), ckv_v[b, pl.ds(j * T, T), :])
            o = acc / jnp.sum(l, axis=-1, keepdims=True)
            for cc in range(4):
                cl_s[pl.ds(pl.multiple_of(cc * 256 + b * 32, 32), 32), :] = o[:, cc * 128:(cc + 1) * 128]
            return carry

        lax.fori_loop(0, B, a_body, 0)

        wait(g_kv[0][1])
        wuv32 = wuv_v.bitcast(U32)
        out_a = jnp.zeros((B, M), F32)
        for h2 in range(H // 2):
            wv_pair = _head_pair(wuv32, h2)
            for p in range(2):
                h = 2 * h2 + p
                cl = jnp.concatenate([cl_s[pl.ds(cc * 256 + h, B, stride=32), :] for cc in range(4)], axis=1)
                ctx = _dot(cl.astype(BF), wv_pair[p])
                out_a = out_a + _dot(ctx.astype(BF), wo_v[pl.ds(h * D, D), :])

        def b_body(b, carry):
            for gb0, g in g_kv[1:]:
                @pl.when(b == gb0)
                def _():
                    wait(g)
            for half in range(2):
                kcat = jnp.concatenate([k_v[b, half * 4 + gi] for gi in range(4)], axis=1)
                s = _dot(qblk_v[b, half], kcat, NT) * SCALE
                m = jnp.max(s, axis=-1, keepdims=True)
                p = jnp.exp(s - m)
                l = jnp.sum(p, axis=-1, keepdims=True)
                pb = p.astype(BF)
                o = None
                for gi in range(4):
                    og = _dot(pb, v_v[b, half * 4 + gi])
                    o = og if o is None else jnp.where(row16 >= 4 * gi, og, o)
                o_s[pl.ds(pl.multiple_of(b * 32 + half * 16, 16), 16), :] = o / l
            return carry

        lax.fori_loop(0, B, b_body, 0)
        for h in range(H):
            ob_v[:, pl.ds(h * D, D)] = o_s[pl.ds(h, B, stride=32), :].astype(BF)

        wait(g_wo)
        omg = 1.0 - gate
        part = gate * out_a + omg * _dot(ob_v[:, pl.ds(0, WO_HEAD * D)], bwo_v[pl.ds(0, WO_HEAD * D), :])

        def t_body(c, part):
            tail_copy(c).wait()
            off = pl.multiple_of((WO_HEAD + c) * D, D)
            return part + omg * _dot(ob_v[:, pl.ds(off, D)], bwo_v[pl.ds(off, D), :])

        part = lax.fori_loop(0, N_TAIL, t_body, part)
        out_v[...] = part.astype(out_v.dtype)
        out_copy.start()

    pl.run_scoped(body, pltpu.SemaphoreType.DMA((N_SEMS,)))
    out_copy.wait()


@jax.jit
def pallas_gated_mix__compressed_kv_cla__sliding_block_cached__decode_kernel(
    A_x: jax.Array,
    A_c_kv: jax.Array,
    A_w_q: jax.Array,
    A_w_uk: jax.Array,
    A_w_uv: jax.Array,
    A_w_o: jax.Array,
    B_x: jax.Array,
    B_k_cache: jax.Array,
    B_v_cache: jax.Array,
    B_wq: jax.Array,
    B_wo: jax.Array,
    gate_w: jax.Array,
):
    assert A_c_kv.shape == (B, SK, DC) and B_k_cache.shape == (B, HKV, SK, D) and A_x.shape == (B, 1, M)
    out = pl.pallas_call(
        _kernel,
        in_specs=[pl.BlockSpec(memory_space=pl.ANY)] * 12,
        out_specs=pl.BlockSpec(memory_space=pl.ANY),
        out_shape=jax.ShapeDtypeStruct((B, M), BF),
        scratch_shapes=[
            pltpu.VMEM((B, M), BF), pltpu.VMEM((B, M), BF), pltpu.VMEM((M,), BF),
            pltpu.VMEM((B, SK, DC), BF),
            pltpu.VMEM((M * H, D), BF), pltpu.VMEM((DC * H, D), BF), pltpu.VMEM((DC * H, D), BF),
            pltpu.VMEM((H * D, M), BF),
            pltpu.VMEM((B, HKV, W, D), BF), pltpu.VMEM((B, HKV, W, D), BF),
            pltpu.VMEM((M, H * D), BF), pltpu.VMEM((H * D, M), BF),
            pltpu.VMEM((4 * 256, 128), F32), pltpu.VMEM((256, 128), F32),
            pltpu.VMEM((B, H, DC), BF), pltpu.VMEM((B, 2, 16, 512), BF),
            pltpu.VMEM((H, SK), F32), pltpu.VMEM((4 * 256, 128), F32),
            pltpu.VMEM((256, 128), F32), pltpu.VMEM((B, H * D), BF), pltpu.VMEM((B, M), BF),
            pltpu.SemaphoreType.DMA(()),
        ],
        compiler_params=pltpu.CompilerParams(vmem_limit_bytes=100 * MiB),
    )(A_x.reshape(B, M), A_c_kv, A_w_q.reshape(M * H, D), A_w_uk.reshape(DC * H, D), A_w_uv.reshape(DC * H, D),
      A_w_o.reshape(H * D, M), B_x.reshape(B, M), B_k_cache, B_v_cache, B_wq, B_wo, gate_w)
    return out.reshape(B, 1, M)
```

```python
import jax
import jax.numpy as jnp
from jax import lax
import jax.experimental.pallas as pl
import jax.experimental.pallas.tpu as pltpu

MiB = 1 << 20
BF = jnp.bfloat16
F32 = jnp.float32
U32 = jnp.uint32
NN = (((1,), (0,)), ((), ()))
NT = (((1,), (1,)), ((), ()))

B, H, D, M, DC, SK = 8, 32, 128, 512, 512, 4096
HKV, W = 8, 1024
SCALE = D ** -0.5

KV_GROUPS = (4, 3, 1)
WO_HEAD = 16
N_TAIL = H - WO_HEAD
STAGE_ROWS = 1024
SEM_W1, SEM_CKV, SEM_W2, SEM_KV = 0, 1, 2, 3
SEM_WO = SEM_KV + len(KV_GROUPS)
N_SEMS = SEM_WO + 1 + N_TAIL


def _dot(a, b, dims=NN):
    return lax.dot_general(a, b, dims, preferred_element_type=F32)


def _head_pair(w32, h2):
    a = w32[pl.ds(h2, 256, stride=32), :]
    b = w32[pl.ds(h2 + 16, 256, stride=32), :]
    lo = (a & jnp.uint32(0xFFFF)) | (b << 16)
    hi = (a >> 16) | (b & jnp.uint32(0xFFFF0000))
    return pltpu.bitcast(lo, BF), pltpu.bitcast(hi, BF)


def _kernel(x_hbm, ckv_hbm, wq_hbm, wuk_hbm, wuv_hbm, wo_hbm, bx_hbm, k_hbm, v_hbm, bwq_hbm, bwo_hbm, g_hbm,
            out_hbm,
            x_v, bx_v, g_v, ckv_v, wq_v, wuk_v, wuv_v, wo_v, k_v, v_v, bwq_v, bwo_v,
            w32_s, q_s, qlat_s, qb_s, ql_v, qblk_v, s_s, cl_s, o_s, ob_v, out_v, out_sem):
    cp = pltpu.make_async_copy
    out_copy = cp(out_v, out_hbm, out_sem)

    def body(sems):
        g_w1 = [cp(wq_hbm, wq_v, sems.at[SEM_W1]), cp(wuk_hbm, wuk_v, sems.at[SEM_W1]),
                cp(bwq_hbm, bwq_v, sems.at[SEM_W1]), cp(x_hbm, x_v, sems.at[SEM_W1]),
                cp(bx_hbm, bx_v, sems.at[SEM_W1]), cp(g_hbm, g_v, sems.at[SEM_W1])]
        g_ckv = [cp(ckv_hbm, ckv_v, sems.at[SEM_CKV])]
        g_w2 = [cp(wuv_hbm, wuv_v, sems.at[SEM_W2]), cp(wo_hbm, wo_v, sems.at[SEM_W2])]
        g_kv = []
        b0 = 0
        for i, n in enumerate(KV_GROUPS):
            sem = sems.at[SEM_KV + i]
            g_kv.append((b0, [cp(k_hbm.at[pl.ds(b0, n), :, pl.ds(SK - W, W)], k_v.at[pl.ds(b0, n)], sem),
                              cp(v_hbm.at[pl.ds(b0, n), :, pl.ds(SK - W, W)], v_v.at[pl.ds(b0, n)], sem)]))
            b0 += n
        g_wo = [cp(bwo_hbm.at[pl.ds(0, WO_HEAD * D)], bwo_v.at[pl.ds(0, WO_HEAD * D)], sems.at[SEM_WO])]

        def tail_copy(c):
            off = pl.multiple_of((WO_HEAD + c) * D, D)
            return cp(bwo_hbm.at[pl.ds(off, D)], bwo_v.at[pl.ds(off, D)], sems.at[SEM_WO + 1 + c])

        def start(g):
            for c in g:
                c.start()

        def wait(g):
            for c in g:
                c.wait()

        start(g_w1)
        start(g_ckv)
        start(g_w2)
        for _, g in g_kv:
            start(g)
        start(g_wo)
        start([tail_copy(c) for c in range(N_TAIL)])

        def stage(w_v):
            def step(i, carry):
                r = pl.multiple_of(i * STAGE_ROWS, STAGE_ROWS)
                r32 = pl.multiple_of(i * (STAGE_ROWS // 2), STAGE_ROWS // 2)
                w32_s[pl.ds(r32, STAGE_ROWS // 2), :] = pltpu.bitcast(w_v[pl.ds(r, STAGE_ROWS), :], U32)
                return carry
            lax.fori_loop(0, M * H // STAGE_ROWS, step, 0)

        wait(g_w1)
        x = x_v[...]
        bx = bx_v[...]
        stage(wq_v)
        for h2 in range(H // 2):
            wq_pair = _head_pair(w32_s, h2)
            for p in range(2):
                q_s[pl.ds((2 * h2 + p) * 8, 8), :] = _dot(x, wq_pair[p])
        stage(wuk_v)
        for h2 in range(H // 2):
            wk_pair = _head_pair(w32_s, h2)
            for p in range(2):
                h = 2 * h2 + p
                q = q_s[pl.ds(h * 8, 8), :].astype(BF)
                ql = _dot(q, wk_pair[p], NT)
                for cc in range(4):
                    qlat_s[pl.ds(cc * 256 + h * 8, 8), :] = ql[:, cc * 128:(cc + 1) * 128]
        for j in range(8):
            qb = _dot(bx, bwq_v[:, j * 512:(j + 1) * 512])
            for r in range(4):
                qb_s[pl.ds((j * 4 + r) * 8, 8), :] = qb[:, r * 128:(r + 1) * 128]
        row16 = lax.broadcasted_iota(jnp.int32, (16, 128), 0)
        for b in range(B):
            parts = [qlat_s[pl.ds(cc * 256 + b, H, stride=8), :] for cc in range(4)]
            ql_v[b] = jnp.concatenate(parts, axis=1).astype(BF)
            qb = qb_s[pl.ds(b, H, stride=8), :]
            for half in range(2):
                qh = qb[half * 16:(half + 1) * 16, :]
                blk = [jnp.where((row16 >= 4 * gi) & (row16 < 4 * gi + 4), qh, 0.0) for gi in range(4)]
                qblk_v[b, half] = jnp.concatenate(blk, axis=1).astype(BF)
        gw = g_v[...].astype(F32).reshape(1, M)
        gate = jax.nn.sigmoid(jnp.sum(x.astype(F32) * gw, axis=-1, keepdims=True))

        T = 1024

        def a_body(b, carry):
            q = ql_v[b]
            mx = None
            for j in range(SK // T):
                s = _dot(q, ckv_v[b, pl.ds(j * T, T), :], NT) * SCALE
                s_s[:, pl.ds(j * T, T)] = s
                for t in range(T // 128):
                    blk = s[:, t * 128:(t + 1) * 128]
                    mx = blk if mx is None else jnp.maximum(mx, blk)
            m = jnp.max(mx, axis=-1, keepdims=True)
            l = jnp.zeros((H, 128), F32)
            acc = jnp.zeros((H, DC), F32)
            for j in range(SK // T):
                p = jnp.exp(s_s[:, pl.ds(j * T, T)] - m)
                for t in range(T // 128):
                    l = l + p[:, t * 128:(t + 1) * 128]
                acc = acc + _dot(p.astype(BF), ckv_v[b, pl.ds(j * T, T), :])
            o = acc / jnp.sum(l, axis=-1, keepdims=True)
            for cc in range(4):
                cl_s[pl.ds(pl.multiple_of(cc * 256 + b * 32, 32), 32), :] = o[:, cc * 128:(cc + 1) * 128]
            return carry

        wait(g_ckv)
        lax.fori_loop(0, B, a_body, 0)

        wait(g_w2)
        stage(wuv_v)
        out_a = jnp.zeros((B, M), F32)
        for h2 in range(H // 2):
            wv_pair = _head_pair(w32_s, h2)
            for p in range(2):
                h = 2 * h2 + p
                cl = jnp.concatenate([cl_s[pl.ds(cc * 256 + h, B, stride=32), :] for cc in range(4)], axis=1)
                ctx = _dot(cl.astype(BF), wv_pair[p])
                out_a = out_a + _dot(ctx.astype(BF), wo_v[pl.ds(h * D, D), :])

        def b_body(b, carry):
            for gb0, g in g_kv:
                @pl.when(b == gb0)
                def _():
                    wait(g)
            for half in range(2):
                kcat = jnp.concatenate([k_v[b, half * 4 + gi] for gi in range(4)], axis=1)
                s = _dot(qblk_v[b, half], kcat, NT) * SCALE
                m = jnp.max(s, axis=-1, keepdims=True)
                p = jnp.exp(s - m)
                l = jnp.sum(p, axis=-1, keepdims=True)
                pb = p.astype(BF)
                o = None
                for gi in range(4):
                    og = _dot(pb, v_v[b, half * 4 + gi])
                    o = og if o is None else jnp.where(row16 >= 4 * gi, og, o)
                o_s[pl.ds(pl.multiple_of(b * 32 + half * 16, 16), 16), :] = o / l
            return carry

        lax.fori_loop(0, B, b_body, 0)
        for h in range(H):
            ob_v[:, pl.ds(h * D, D)] = o_s[pl.ds(h, B, stride=32), :].astype(BF)

        wait(g_wo)
        omg = 1.0 - gate
        part = gate * out_a + omg * _dot(ob_v[:, pl.ds(0, WO_HEAD * D)], bwo_v[pl.ds(0, WO_HEAD * D), :])

        def t_body(c, part):
            tail_copy(c).wait()
            off = pl.multiple_of((WO_HEAD + c) * D, D)
            return part + omg * _dot(ob_v[:, pl.ds(off, D)], bwo_v[pl.ds(off, D), :])

        part = lax.fori_loop(0, N_TAIL, t_body, part)
        out_v[...] = part.astype(out_v.dtype)
        out_copy.start()

    pl.run_scoped(body, pltpu.SemaphoreType.DMA((N_SEMS,)))
    out_copy.wait()


@jax.jit
def pallas_gated_mix__compressed_kv_cla__sliding_block_cached__decode_kernel(
    A_x: jax.Array,
    A_c_kv: jax.Array,
    A_w_q: jax.Array,
    A_w_uk: jax.Array,
    A_w_uv: jax.Array,
    A_w_o: jax.Array,
    B_x: jax.Array,
    B_k_cache: jax.Array,
    B_v_cache: jax.Array,
    B_wq: jax.Array,
    B_wo: jax.Array,
    gate_w: jax.Array,
):
    assert A_c_kv.shape == (B, SK, DC) and B_k_cache.shape == (B, HKV, SK, D) and A_x.shape == (B, 1, M)
    out = pl.pallas_call(
        _kernel,
        in_specs=[pl.BlockSpec(memory_space=pl.ANY)] * 12,
        out_specs=pl.BlockSpec(memory_space=pl.ANY),
        out_shape=jax.ShapeDtypeStruct((B, M), BF),
        scratch_shapes=[
            pltpu.VMEM((B, M), BF), pltpu.VMEM((B, M), BF), pltpu.VMEM((M,), BF),
            pltpu.VMEM((B, SK, DC), BF),
            pltpu.VMEM((M * H, D), BF), pltpu.VMEM((DC * H, D), BF), pltpu.VMEM((DC * H, D), BF),
            pltpu.VMEM((H * D, M), BF),
            pltpu.VMEM((B, HKV, W, D), BF), pltpu.VMEM((B, HKV, W, D), BF),
            pltpu.VMEM((M, H * D), BF), pltpu.VMEM((H * D, M), BF),
            pltpu.VMEM((M * H // 2, D), U32), pltpu.VMEM((H * B, D), F32),
            pltpu.VMEM((4 * 256, 128), F32), pltpu.VMEM((256, 128), F32),
            pltpu.VMEM((B, H, DC), BF), pltpu.VMEM((B, 2, 16, 512), BF),
            pltpu.VMEM((H, SK), F32), pltpu.VMEM((4 * 256, 128), F32),
            pltpu.VMEM((256, 128), F32), pltpu.VMEM((B, H * D), BF), pltpu.VMEM((B, M), BF),
            pltpu.SemaphoreType.DMA(()),
        ],
        compiler_params=pltpu.CompilerParams(vmem_limit_bytes=110 * MiB),
    )(A_x.reshape(B, M), A_c_kv, A_w_q.reshape(M * H, D), A_w_uk.reshape(DC * H, D), A_w_uv.reshape(DC * H, D),
      A_w_o.reshape(H * D, M), B_x.reshape(B, M), B_k_cache, B_v_cache, B_wq, B_wo, gate_w)
    return out.reshape(B, 1, M)
```

```python
import jax
import jax.numpy as jnp
from jax import lax
import jax.experimental.pallas as pl
import jax.experimental.pallas.tpu as pltpu

MiB = 1 << 20
BF = jnp.bfloat16
F32 = jnp.float32
U32 = jnp.uint32
NN = (((1,), (0,)), ((), ()))
NT = (((1,), (1,)), ((), ()))

B, H, D, M, DC, SK = 8, 32, 128, 512, 512, 4096
HKV, W = 8, 1024
SCALE = D ** -0.5

KV_GROUPS = (4, 3, 1)
WO_HEAD = 16
N_TAIL = H - WO_HEAD
STAGE_ROWS = 1024
SEM_W1, SEM_CKV, SEM_W2, SEM_KV = 0, 1, 2, 3
SEM_WO = SEM_KV + len(KV_GROUPS)
N_SEMS = SEM_WO + 1 + N_TAIL


def _dot(a, b, dims=NN):
    return lax.dot_general(a, b, dims, preferred_element_type=F32)


def _head_pair(w32, h2):
    a = w32[pl.ds(h2, 256, stride=32), :]
    b = w32[pl.ds(h2 + 16, 256, stride=32), :]
    lo = (a & jnp.uint32(0xFFFF)) | (b << 16)
    hi = (a >> 16) | (b & jnp.uint32(0xFFFF0000))
    return pltpu.bitcast(lo, BF), pltpu.bitcast(hi, BF)


def _kernel(x_hbm, ckv_hbm, wq_hbm, wuk_hbm, wuv_hbm, wo_hbm, k_hbm, v_hbm, bwq_hbm, bwo_hbm, g_hbm,
            out_hbm,
            x_v, g_v, ckv_v, wq_v, wuk_v, wuv_v, wo_v, k_v, v_v, bwq_v, bwo_v,
            w32_s, q_s, qlat_s, qb_s, ql_v, qblk_v, s_s, cl_s, o_s, ob_v, out_v, out_sem):
    cp = pltpu.make_async_copy
    out_copy = cp(out_v, out_hbm, out_sem)

    def body(sems):
        g_w1 = [cp(wq_hbm, wq_v, sems.at[SEM_W1]), cp(wuk_hbm, wuk_v, sems.at[SEM_W1]),
                cp(bwq_hbm, bwq_v, sems.at[SEM_W1]), cp(x_hbm, x_v, sems.at[SEM_W1]),
                cp(g_hbm, g_v, sems.at[SEM_W1])]
        g_ckv = [cp(ckv_hbm, ckv_v, sems.at[SEM_CKV])]
        g_w2 = [cp(wuv_hbm, wuv_v, sems.at[SEM_W2]), cp(wo_hbm, wo_v, sems.at[SEM_W2])]
        g_kv = []
        b0 = 0
        for i, n in enumerate(KV_GROUPS):
            sem = sems.at[SEM_KV + i]
            g_kv.append((b0, [cp(k_hbm.at[pl.ds(b0, n), :, pl.ds(SK - W, W)], k_v.at[pl.ds(b0, n)], sem),
                              cp(v_hbm.at[pl.ds(b0, n), :, pl.ds(SK - W, W)], v_v.at[pl.ds(b0, n)], sem)]))
            b0 += n
        g_wo = [cp(bwo_hbm.at[pl.ds(0, WO_HEAD * D)], bwo_v.at[pl.ds(0, WO_HEAD * D)], sems.at[SEM_WO])]

        def tail_copy(c):
            off = pl.multiple_of((WO_HEAD + c) * D, D)
            return cp(bwo_hbm.at[pl.ds(off, D)], bwo_v.at[pl.ds(off, D)], sems.at[SEM_WO + 1 + c])

        def start(g):
            for c in g:
                c.start()

        def wait(g):
            for c in g:
                c.wait()

        start(g_w1)
        start(g_ckv)
        start(g_w2)
        for _, g in g_kv:
            start(g)
        start(g_wo)
        start([tail_copy(c) for c in range(N_TAIL)])

        def stage(w_v):
            def step(i, carry):
                r = pl.multiple_of(i * STAGE_ROWS, STAGE_ROWS)
                r32 = pl.multiple_of(i * (STAGE_ROWS // 2), STAGE_ROWS // 2)
                w32_s[pl.ds(r32, STAGE_ROWS // 2), :] = pltpu.bitcast(w_v[pl.ds(r, STAGE_ROWS), :], U32)
                return carry
            lax.fori_loop(0, M * H // STAGE_ROWS, step, 0)

        wait(g_w1)
        x = x_v[...]
        stage(wq_v)
        for h2 in range(H // 2):
            wq_pair = _head_pair(w32_s, h2)
            for p in range(2):
                q_s[pl.ds((2 * h2 + p) * 8, 8), :] = _dot(x, wq_pair[p])
        stage(wuk_v)
        for h2 in range(H // 2):
            wk_pair = _head_pair(w32_s, h2)
            for p in range(2):
                h = 2 * h2 + p
                q = q_s[pl.ds(h * 8, 8), :].astype(BF)
                ql = _dot(q, wk_pair[p], NT)
                for cc in range(4):
                    qlat_s[pl.ds(cc * 256 + h * 8, 8), :] = ql[:, cc * 128:(cc + 1) * 128]
        for j in range(8):
            qb = _dot(x, bwq_v[:, j * 512:(j + 1) * 512])
            for r in range(4):
                qb_s[pl.ds((j * 4 + r) * 8, 8), :] = qb[:, r * 128:(r + 1) * 128]
        row16 = lax.broadcasted_iota(jnp.int32, (16, 128), 0)
        for b in range(B):
            parts = [qlat_s[pl.ds(cc * 256 + b, H, stride=8), :] for cc in range(4)]
            ql_v[b] = jnp.concatenate(parts, axis=1).astype(BF)
            qb = qb_s[pl.ds(b, H, stride=8), :]
            for half in range(2):
                qh = qb[half * 16:(half + 1) * 16, :]
                blk = [jnp.where((row16 >= 4 * gi) & (row16 < 4 * gi + 4), qh, 0.0) for gi in range(4)]
                qblk_v[b, half] = jnp.concatenate(blk, axis=1).astype(BF)
        gw = g_v[...].astype(F32).reshape(1, M)
        gate = jax.nn.sigmoid(jnp.sum(x.astype(F32) * gw, axis=-1, keepdims=True))

        T = 1024

        def a_body(b, carry):
            q = ql_v[b]
            mx = None
            for j in range(SK // T):
                s = _dot(q, ckv_v[b, pl.ds(j * T, T), :], NT) * SCALE
                s_s[:, pl.ds(j * T, T)] = s
                for t in range(T // 128):
                    blk = s[:, t * 128:(t + 1) * 128]
                    mx = blk if mx is None else jnp.maximum(mx, blk)
            m = jnp.max(mx, axis=-1, keepdims=True)
            l = jnp.zeros((H, 128), F32)
            acc = jnp.zeros((H, DC), F32)
            for j in range(SK // T):
                p = jnp.exp(s_s[:, pl.ds(j * T, T)] - m)
                for t in range(T // 128):
                    l = l + p[:, t * 128:(t + 1) * 128]
                acc = acc + _dot(p.astype(BF), ckv_v[b, pl.ds(j * T, T), :])
            o = acc / jnp.sum(l, axis=-1, keepdims=True)
            for cc in range(4):
                cl_s[pl.ds(pl.multiple_of(cc * 256 + b * 32, 32), 32), :] = o[:, cc * 128:(cc + 1) * 128]
            return carry

        wait(g_ckv)
        lax.fori_loop(0, B, a_body, 0)

        wait(g_w2)
        stage(wuv_v)
        out_a = jnp.zeros((B, M), F32)
        for h2 in range(H // 2):
            wv_pair = _head_pair(w32_s, h2)
            for p in range(2):
                h = 2 * h2 + p
                cl = jnp.concatenate([cl_s[pl.ds(cc * 256 + h, B, stride=32), :] for cc in range(4)], axis=1)
                ctx = _dot(cl.astype(BF), wv_pair[p])
                out_a = out_a + _dot(ctx.astype(BF), wo_v[pl.ds(h * D, D), :])

        def b_body(b, carry):
            for gb0, g in g_kv:
                @pl.when(b == gb0)
                def _():
                    wait(g)
            for half in range(2):
                kcat = jnp.concatenate([k_v[b, half * 4 + gi] for gi in range(4)], axis=1)
                s = _dot(qblk_v[b, half], kcat, NT) * SCALE
                m = jnp.max(s, axis=-1, keepdims=True)
                p = jnp.exp(s - m)
                l = jnp.sum(p, axis=-1, keepdims=True)
                pb = p.astype(BF)
                o = None
                for gi in range(4):
                    og = _dot(pb, v_v[b, half * 4 + gi])
                    o = og if o is None else jnp.where(row16 >= 4 * gi, og, o)
                o_s[pl.ds(pl.multiple_of(b * 32 + half * 16, 16), 16), :] = o / l
            return carry

        lax.fori_loop(0, B, b_body, 0)
        for h in range(H):
            ob_v[:, pl.ds(h * D, D)] = o_s[pl.ds(h, B, stride=32), :].astype(BF)

        wait(g_wo)
        omg = 1.0 - gate
        part = gate * out_a + omg * _dot(ob_v[:, pl.ds(0, WO_HEAD * D)], bwo_v[pl.ds(0, WO_HEAD * D), :])

        def t_body(c, part):
            tail_copy(c).wait()
            off = pl.multiple_of((WO_HEAD + c) * D, D)
            return part + omg * _dot(ob_v[:, pl.ds(off, D)], bwo_v[pl.ds(off, D), :])

        part = lax.fori_loop(0, N_TAIL, t_body, part)
        out_v[...] = part.astype(out_v.dtype)
        out_copy.start()

    pl.run_scoped(body, pltpu.SemaphoreType.DMA((N_SEMS,)))
    out_copy.wait()


@jax.jit
def pallas_gated_mix__compressed_kv_cla__sliding_block_cached__decode_kernel(
    A_x: jax.Array,
    A_c_kv: jax.Array,
    A_w_q: jax.Array,
    A_w_uk: jax.Array,
    A_w_uv: jax.Array,
    A_w_o: jax.Array,
    B_x: jax.Array,
    B_k_cache: jax.Array,
    B_v_cache: jax.Array,
    B_wq: jax.Array,
    B_wo: jax.Array,
    gate_w: jax.Array,
):
    del B_x
    assert A_c_kv.shape == (B, SK, DC) and B_k_cache.shape == (B, HKV, SK, D) and A_x.shape == (B, 1, M)
    out = pl.pallas_call(
        _kernel,
        in_specs=[pl.BlockSpec(memory_space=pl.ANY)] * 11,
        out_specs=pl.BlockSpec(memory_space=pl.ANY),
        out_shape=jax.ShapeDtypeStruct((B, M), BF),
        scratch_shapes=[
            pltpu.VMEM((B, M), BF), pltpu.VMEM((M,), BF),
            pltpu.VMEM((B, SK, DC), BF),
            pltpu.VMEM((M * H, D), BF), pltpu.VMEM((DC * H, D), BF), pltpu.VMEM((DC * H, D), BF),
            pltpu.VMEM((H * D, M), BF),
            pltpu.VMEM((B, HKV, W, D), BF), pltpu.VMEM((B, HKV, W, D), BF),
            pltpu.VMEM((M, H * D), BF), pltpu.VMEM((H * D, M), BF),
            pltpu.VMEM((M * H // 2, D), U32), pltpu.VMEM((H * B, D), F32),
            pltpu.VMEM((4 * 256, 128), F32), pltpu.VMEM((256, 128), F32),
            pltpu.VMEM((B, H, DC), BF), pltpu.VMEM((B, 2, 16, 512), BF),
            pltpu.VMEM((H, SK), F32), pltpu.VMEM((4 * 256, 128), F32),
            pltpu.VMEM((256, 128), F32), pltpu.VMEM((B, H * D), BF), pltpu.VMEM((B, M), BF),
            pltpu.SemaphoreType.DMA(()),
        ],
        compiler_params=pltpu.CompilerParams(vmem_limit_bytes=110 * MiB),
    )(A_x.reshape(B, M), A_c_kv, A_w_q.reshape(M * H, D), A_w_uk.reshape(DC * H, D), A_w_uv.reshape(DC * H, D),
      A_w_o.reshape(H * D, M), B_k_cache, B_v_cache, B_wq, B_wo, gate_w)
    return out.reshape(B, 1, M)
```

```python
import jax
import jax.numpy as jnp
from jax import lax
import jax.experimental.pallas as pl
import jax.experimental.pallas.tpu as pltpu

MiB = 1 << 20
BF = jnp.bfloat16
F32 = jnp.float32
U32 = jnp.uint32
NN = (((1,), (0,)), ((), ()))
NT = (((1,), (1,)), ((), ()))

B, H, D, M, DC, SK = 8, 32, 128, 512, 512, 4096
HKV, W = 8, 1024
SCALE = D ** -0.5

KV_GROUPS = (4, 3, 1)
WO_HEAD = 16
N_TAIL = H - WO_HEAD
STAGE_ROWS = 1024
SEM_W1, SEM_CKV, SEM_W2, SEM_KV = 0, 1, 2, 3
SEM_WO = SEM_KV + len(KV_GROUPS)
N_SEMS = SEM_WO + 1 + N_TAIL


def _dot(a, b, dims=NN):
    return lax.dot_general(a, b, dims, preferred_element_type=F32)


def _head_pair(w32, h2):
    a = w32[pl.ds(h2, 256, stride=32), :]
    b = w32[pl.ds(h2 + 16, 256, stride=32), :]
    lo = (a & jnp.uint32(0xFFFF)) | (b << 16)
    hi = (a >> 16) | (b & jnp.uint32(0xFFFF0000))
    return pltpu.bitcast(lo, BF), pltpu.bitcast(hi, BF)


def _kernel(x_hbm, ckv_hbm, wq_hbm, wuk_hbm, wuv_hbm, wo_hbm, k_hbm, v_hbm, bwq_hbm, bwo_hbm, g_hbm,
            out_hbm,
            x_v, g_v, ckv_v, wq_v, wuk_v, wuv_v, wo_v, k_v, v_v, bwq_v, bwo_v,
            w32_s, q_s, qlat_s, qb_s, ql_v, qblk_v, s_s, cl_s, o_s, ob_v, out_v, out_sem):
    cp = pltpu.make_async_copy
    out_copy = cp(out_v, out_hbm, out_sem)

    def body(sems):
        g_w1 = [cp(wq_hbm, wq_v, sems.at[SEM_W1]), cp(wuk_hbm, wuk_v, sems.at[SEM_W1]),
                cp(bwq_hbm, bwq_v, sems.at[SEM_W1]), cp(x_hbm, x_v, sems.at[SEM_W1]),
                cp(g_hbm, g_v, sems.at[SEM_W1])]
        g_ckv = [cp(ckv_hbm, ckv_v, sems.at[SEM_CKV])]
        g_w2 = [cp(wuv_hbm, wuv_v, sems.at[SEM_W2]), cp(wo_hbm, wo_v, sems.at[SEM_W2])]
        g_kv = []
        b0 = 0
        for i, n in enumerate(KV_GROUPS):
            sem = sems.at[SEM_KV + i]
            g_kv.append((b0, [cp(k_hbm.at[pl.ds(b0, n), :, pl.ds(SK - W, W)], k_v.at[pl.ds(b0, n)], sem),
                              cp(v_hbm.at[pl.ds(b0, n), :, pl.ds(SK - W, W)], v_v.at[pl.ds(b0, n)], sem)]))
            b0 += n
        g_wo = [cp(bwo_hbm.at[pl.ds(0, WO_HEAD * D)], bwo_v.at[pl.ds(0, WO_HEAD * D)], sems.at[SEM_WO])]

        def tail_copy(c):
            off = pl.multiple_of((WO_HEAD + c) * D, D)
            return cp(bwo_hbm.at[pl.ds(off, D)], bwo_v.at[pl.ds(off, D)], sems.at[SEM_WO + 1 + c])

        def start(g):
            for c in g:
                c.start()

        def wait(g):
            for c in g:
                c.wait()

        start(g_w1)
        start(g_ckv)
        start(g_w2)
        for _, g in g_kv:
            start(g)
        start(g_wo)
        start([tail_copy(c) for c in range(N_TAIL)])

        def stage(w_v):
            def step(i, carry):
                r = pl.multiple_of(i * STAGE_ROWS, STAGE_ROWS)
                r32 = pl.multiple_of(i * (STAGE_ROWS // 2), STAGE_ROWS // 2)
                w32_s[pl.ds(r32, STAGE_ROWS // 2), :] = pltpu.bitcast(w_v[pl.ds(r, STAGE_ROWS), :], U32)
                return carry
            lax.fori_loop(0, M * H // STAGE_ROWS, step, 0)

        wait(g_w1)
        x = x_v[...]
        stage(wq_v)
        for h2 in range(H // 2):
            wq_pair = _head_pair(w32_s, h2)
            for p in range(2):
                q_s[pl.ds((2 * h2 + p) * 8, 8), :] = _dot(x, wq_pair[p])
        stage(wuk_v)
        for h2 in range(H // 2):
            wk_pair = _head_pair(w32_s, h2)
            for p in range(2):
                h = 2 * h2 + p
                q = q_s[pl.ds(h * 8, 8), :].astype(BF)
                ql = _dot(q, wk_pair[p], NT)
                for cc in range(4):
                    qlat_s[pl.ds(cc * 256 + h * 8, 8), :] = ql[:, cc * 128:(cc + 1) * 128]
        for j in range(8):
            qb = _dot(x, bwq_v[:, j * 512:(j + 1) * 512])
            for r in range(4):
                qb_s[pl.ds((j * 4 + r) * 8, 8), :] = qb[:, r * 128:(r + 1) * 128]
        row16 = lax.broadcasted_iota(jnp.int32, (16, 128), 0)
        for b in range(B):
            parts = [qlat_s[pl.ds(cc * 256 + b, H, stride=8), :] for cc in range(4)]
            ql_v[b] = jnp.concatenate(parts, axis=1).astype(BF)
            qb = qb_s[pl.ds(b, H, stride=8), :]
            for half in range(2):
                qh = qb[half * 16:(half + 1) * 16, :]
                blk = [jnp.where((row16 >= 4 * gi) & (row16 < 4 * gi + 4), qh, 0.0) for gi in range(4)]
                qblk_v[b, half] = jnp.concatenate(blk, axis=1).astype(BF)
        gw = g_v[...].astype(F32).reshape(1, M)
        gate = jax.nn.sigmoid(jnp.sum(x.astype(F32) * gw, axis=-1, keepdims=True))

        T = 1024

        def a_body(b, carry):
            q = ql_v[b]
            mx = None
            for j in range(SK // T):
                s = _dot(q, ckv_v[b, pl.ds(j * T, T), :], NT) * SCALE
                s_s[:, pl.ds(j * T, T)] = s
                for t in range(T // 128):
                    blk = s[:, t * 128:(t + 1) * 128]
                    mx = blk if mx is None else jnp.maximum(mx, blk)
            m = jnp.max(mx, axis=-1, keepdims=True)
            l = jnp.zeros((H, 128), F32)
            acc = jnp.zeros((H, DC), F32)
            for j in range(SK // T):
                p = jnp.exp(s_s[:, pl.ds(j * T, T)] - m)
                for t in range(T // 128):
                    l = l + p[:, t * 128:(t + 1) * 128]
                acc = acc + _dot(p.astype(BF), ckv_v[b, pl.ds(j * T, T), :])
            o = acc / jnp.sum(l, axis=-1, keepdims=True)
            for cc in range(4):
                cl_s[pl.ds(pl.multiple_of(cc * 256 + b * 32, 32), 32), :] = o[:, cc * 128:(cc + 1) * 128]
            return carry

        wait(g_ckv)
        lax.fori_loop(0, B, a_body, 0)

        wait(g_w2)
        stage(wuv_v)
        out_a = jnp.zeros((B, M), F32)
        for h2 in range(H // 2):
            wv_pair = _head_pair(w32_s, h2)
            for p in range(2):
                h = 2 * h2 + p
                cl = jnp.concatenate([cl_s[pl.ds(cc * 256 + h, B, stride=32), :] for cc in range(4)], axis=1)
                ctx = _dot(cl.astype(BF), wv_pair[p])
                out_a = out_a + _dot(ctx.astype(BF), wo_v[pl.ds(h * D, D), :])

        def b_body(b, carry):
            for gb0, g in g_kv:
                @pl.when(b == gb0)
                def _():
                    wait(g)
            for half in range(2):
                kcat = jnp.concatenate([k_v[b, half * 4 + gi] for gi in range(4)], axis=1)
                s = _dot(qblk_v[b, half], kcat, NT) * SCALE
                m = jnp.max(s, axis=-1, keepdims=True)
                p = jnp.exp(s - m)
                l = jnp.sum(p, axis=-1, keepdims=True)
                pb = p.astype(BF)
                o = None
                for gi in range(4):
                    og = _dot(pb, v_v[b, half * 4 + gi])
                    o = og if o is None else jnp.where(row16 >= 4 * gi, og, o)
                o_s[pl.ds(pl.multiple_of(b * 32 + half * 16, 16), 16), :] = o / l
            return carry

        lax.fori_loop(0, B, b_body, 0)
        for h in range(H):
            ob_v[:, pl.ds(h * D, D)] = o_s[pl.ds(h, B, stride=32), :].astype(BF)

        wait(g_wo)
        omg = 1.0 - gate
        part = gate * out_a + omg * _dot(ob_v[:, pl.ds(0, WO_HEAD * D)], bwo_v[pl.ds(0, WO_HEAD * D), :])

        def t_body(c, part):
            tail_copy(c).wait()
            off = pl.multiple_of((WO_HEAD + c) * D, D)
            return part + omg * _dot(ob_v[:, pl.ds(off, D)], bwo_v[pl.ds(off, D), :])

        part = lax.fori_loop(0, N_TAIL, t_body, part)
        out_v[...] = part.astype(out_v.dtype)
        out_copy.start()

    pl.run_scoped(body, pltpu.SemaphoreType.DMA((N_SEMS,)))
    out_copy.wait()


@jax.jit
def pallas_gated_mix__compressed_kv_cla__sliding_block_cached__decode_kernel(
    A_x: jax.Array,
    A_c_kv: jax.Array,
    A_w_q: jax.Array,
    A_w_uk: jax.Array,
    A_w_uv: jax.Array,
    A_w_o: jax.Array,
    B_x: jax.Array,
    B_k_cache: jax.Array,
    B_v_cache: jax.Array,
    B_wq: jax.Array,
    B_wo: jax.Array,
    gate_w: jax.Array,
):
    del B_x
    assert A_c_kv.shape == (B, SK, DC) and B_k_cache.shape == (B, HKV, SK, D) and A_x.shape == (B, 1, M)
    out = pl.pallas_call(
        _kernel,
        in_specs=[pl.BlockSpec(memory_space=pl.ANY)] * 11,
        out_specs=pl.BlockSpec(memory_space=pl.ANY),
        out_shape=jax.ShapeDtypeStruct((B, M), BF),
        scratch_shapes=[
            pltpu.VMEM((B, M), BF), pltpu.VMEM((M,), BF),
            pltpu.VMEM((B, SK, DC), BF),
            pltpu.VMEM((M * H, D), BF), pltpu.VMEM((DC * H, D), BF), pltpu.VMEM((DC * H, D), BF),
            pltpu.VMEM((H * D, M), BF),
            pltpu.VMEM((B, HKV, W, D), BF), pltpu.VMEM((B, HKV, W, D), BF),
            pltpu.VMEM((M, H * D), BF), pltpu.VMEM((H * D, M), BF),
            pltpu.VMEM((M * H // 2 + 32, D), U32), pltpu.VMEM((H * B, D), F32),
            pltpu.VMEM((4 * 256 + 32, 128), F32), pltpu.VMEM((256 + 32, 128), F32),
            pltpu.VMEM((B, H, DC), BF), pltpu.VMEM((B, 2, 16, 512), BF),
            pltpu.VMEM((H, SK), F32), pltpu.VMEM((4 * 256 + 32, 128), F32),
            pltpu.VMEM((256 + 32, 128), F32), pltpu.VMEM((B, H * D), BF), pltpu.VMEM((B, M), BF),
            pltpu.SemaphoreType.DMA(()),
        ],
        compiler_params=pltpu.CompilerParams(vmem_limit_bytes=110 * MiB),
    )(A_x.reshape(B, M), A_c_kv, A_w_q.reshape(M * H, D), A_w_uk.reshape(DC * H, D), A_w_uv.reshape(DC * H, D),
      A_w_o.reshape(H * D, M), B_k_cache, B_v_cache, B_wq, B_wo, gate_w)
    return out.reshape(B, 1, M)
```
